```python
import jax
import jax.numpy as jnp

def _softmax(x, axis=-1):
    return jax.nn.softmax(x, axis=axis)
def _gelu(x):
    return jax.nn.gelu(x, approximate=True)
def _silu(x):
    return jax.nn.silu(x)
def _sigmoid(x):
    return jax.nn.sigmoid(x)
def _layernorm(x, axis=-1, eps=1e-5):
    m = jnp.mean(x, axis=axis, keepdims=True)
    v = jnp.var(x, axis=axis, keepdims=True)
    return (x - m) / jnp.sqrt(v + eps)
def _scatter_add(tgt, idx, src, axis=0):
    return tgt.at[idx].add(src)
def _segment_sum(src, seg, n):
    return jax.ops.segment_sum(src, seg, n)
class _Rng:
    def __init__(self, key):
        self._k = key
    def _next(self):
        self._k, sub = jax.random.split(self._k)
        return sub
    def normal(self, shape):
        return jax.random.normal(self._next(), shape, dtype=jnp.bfloat16)
    def randint(self, lo, hi, shape):
        return jax.random.randint(self._next(), shape, lo, hi, dtype=jnp.int32)
    def uniform(self, shape, lo=0.0, hi=1.0):
        return jax.random.uniform(self._next(), shape, jnp.bfloat16, lo, hi)
    def permutation(self, n):
        return jax.random.permutation(self._next(), n)


kernel_name = 'standalone__layernorm_linear__prompt'

def setup_inputs():
    _rng = _Rng(jax.random.key(int.from_bytes(__import__("os").urandom(4), "little")))
    _w = (lambda a: (lambda t: t.astype(jnp.bfloat16) if jnp.issubdtype(t.dtype, jnp.floating) else t)(jnp.asarray(a)))
    B, S, D = 2, 2048, 1024
    return {
        "x": _w((lambda *s: _rng.normal(s) * 0.05)(B, S, D)),
        "g": _w((lambda *s: _rng.normal(s) * 0.05)(D) + 1.0),
        "b": _w((lambda *s: _rng.normal(s) * 0.05)(D)),
        "w": _w((lambda *s: _rng.normal(s) * 0.05)(D, D)),
    }

def reference(x, g, b, w):
    return (_layernorm(x, axis=-1) * g + b) @ w
```

```python
import jax
import jax.numpy as jnp
from jax import lax
import jax.experimental.pallas as pl
import jax.experimental.pallas.tpu as pltpu

_EPS = 1e-5
_BLK = 128
_GRP = 16
_P = 4
_U = 4


def _kernel(x_hbm, g_hbm, b_hbm, w_hbm, o_hbm,
            xo, wbuf, ybuf, g16, b16, gb, sem_in, sem_o, *, M, D):
    NB = M // _BLK
    NT = D // _BLK
    GPB = _BLK // _GRP
    y32 = ybuf.bitcast(jnp.uint32)
    w32 = wbuf.bitcast(jnp.uint32)
    LASTQ = GPB * NB - 1
    DUMMYQ = GPB * NB + GPB
    xahead = _U + 2

    def xcopy(i):
        r = pl.multiple_of(i * _BLK, _BLK)
        return pltpu.make_async_copy(
            x_hbm.at[pl.ds(r, _BLK), :], xo.at[pl.ds(r, _BLK), :], sem_in.at[i])

    def wcopy(j):
        c = pl.multiple_of(j * _BLK, _BLK)
        return pltpu.make_async_copy(
            w_hbm.at[:, pl.ds(c, _BLK)], wbuf.at[j], sem_in.at[NB + j])

    def gcopy():
        return pltpu.make_async_copy(g_hbm, g16, sem_in.at[NB + NT])

    def bcopy():
        return pltpu.make_async_copy(b_hbm, b16, sem_in.at[NB + NT + 1])

    def ocopy(i, nt):
        r = pl.multiple_of(i * _BLK, _BLK)
        c = pl.multiple_of(nt * _BLK, _BLK)
        return pltpu.make_async_copy(
            xo.at[pl.ds(r, _BLK), pl.ds(c, _BLK)],
            o_hbm.at[pl.ds(r, _BLK), pl.ds(c, _BLK)], sem_o)

    def ln_load(q):
        return xo[pl.ds(pl.multiple_of(q * _GRP, _GRP), _GRP), :]

    def ln_stats(q):
        x = ln_load(q).astype(jnp.float32)
        mean = jnp.mean(x, axis=-1, keepdims=True)
        var = jnp.maximum(
            jnp.mean(x * x, axis=-1, keepdims=True) - mean * mean, 0.0)
        rstd = lax.rsqrt(var + _EPS)
        return (jnp.broadcast_to(rstd, (_GRP, _BLK)),
                jnp.broadcast_to(mean, (_GRP, _BLK)))

    def ln_apply(q, xb, stats):
        rstd, mean = stats
        yv = ybuf.at[:, pl.ds(pl.multiple_of(q * _GRP, _GRP), _GRP), :]
        x = xb.astype(jnp.float32)
        for kt in range(NT):
            cols = slice(kt * _BLK, (kt + 1) * _BLK)
            y = (x[:, cols] - mean) * rstd * gb[0:1, cols] + gb[1:2, cols]
            yv[kt] = y.astype(jnp.bfloat16)

    def ln_block(blk):
        for grp in range(GPB):
            q = GPB * blk + grp
            ln_apply(q, ln_load(q), ln_stats(q))

    def step(blk, nt, mid=None, post=None):
        yv = y32.at[:, pl.ds(pl.multiple_of(blk * (_BLK // 2), _BLK // 2), _BLK // 2), :]
        lhs = jnp.concatenate(
            [pltpu.bitcast(yv[kt], jnp.bfloat16) for kt in range(NT)], axis=1)
        rhs = pltpu.bitcast(w32[nt], jnp.bfloat16)
        acc = jnp.dot(lhs, rhs, preferred_element_type=jnp.float32)
        held = mid() if mid is not None else None
        ov = xo.at[pl.ds(pl.multiple_of(blk * _BLK, _BLK), _BLK), :]
        ov[:, pl.ds(pl.multiple_of(nt * _BLK, _BLK), _BLK)] = acc.astype(jnp.bfloat16)
        ocopy(blk, nt).start()
        if post is not None:
            post(held)
        return held

    def ln_step(blk, nt, q_apply_load, q_apply_store, q_stats, stats):
        held = step(
            blk, nt,
            mid=lambda: (ln_load(q_apply_load), ln_stats(q_stats)),
            post=lambda h: ln_apply(q_apply_store, h[0], stats))
        return held[1]

    nslots = GPB + 1
    s0 = (NT - 1) * _P - nslots
    nt0 = 1 + s0 // _P
    xcopy(0).start()
    gcopy().start()
    bcopy().start()
    wcopy(0).start()
    for i in range(1, _P):
        xcopy(i).start()
    for j in range(1, NT):
        if j == nt0 + 1:
            xcopy(_P).start()
        wcopy(j).start()
    for i in range(_P + 1, _P + xahead):
        xcopy(i).start()

    xcopy(0).wait()
    gcopy().wait()
    bcopy().wait()
    gb[0:1, :] = g16[...].astype(jnp.float32).reshape(1, D)
    gb[1:2, :] = b16[...].astype(jnp.float32).reshape(1, D)
    ln_block(0)
    wcopy(0).wait()
    for i in range(_P):
        if i > 0:
            xcopy(i).wait()
            ln_block(i)
        step(i, 0)

    def startup(nt, stats):
        wcopy(nt).wait()

        @pl.when(nt == nt0 - 1)
        def _():
            xcopy(_P).wait()

        @pl.when(nt == NT - 1)
        def _():
            xcopy(_P + 1).wait()

        for i in range(_P):
            s = (nt - 1) * _P + i - s0
            act = s >= 0
            stats = ln_step(
                i, nt,
                jnp.where(act, GPB * _P + s, 0),
                jnp.where(act, GPB * _P + s, DUMMYQ),
                jnp.where(s + 1 >= 0, jnp.minimum(GPB * _P + s + 1, GPB * _P + GPB), 0),
                stats)
        return stats

    zero = jnp.zeros((_GRP, _BLK), jnp.float32)
    lax.fori_loop(1, NT, startup, (zero, zero))

    def main(j, stats):
        b0 = _P + j * _U
        for k in range(_U):
            @pl.when(b0 + 2 + k < NB)
            def _():
                xcopy(b0 + 2 + k).wait()
        for k in range(_U):
            @pl.when(b0 + xahead + k < NB)
            def _():
                xcopy(b0 + xahead + k).start()
        for k in range(_U):
            blk = b0 + k
            for nt in range(NT):
                q = GPB * (blk + 1) + nt + 1
                stats = ln_step(blk, nt, jnp.minimum(q, LASTQ), q,
                                jnp.minimum(q + 1, LASTQ), stats)
        return stats

    lax.fori_loop(0, (NB - _P) // _U, main, ln_stats(GPB * (_P + 1) + 1))

    pltpu.make_async_copy(xo, o_hbm, sem_o).wait()


@jax.jit
def pallas_standalone__layernorm_linear__prompt_kernel(
    x: jax.Array,
    g: jax.Array,
    b: jax.Array,
    w: jax.Array,
):
    B, S, D = x.shape
    M = B * S
    NB = M // _BLK
    NT = D // _BLK
    any_spec = pl.BlockSpec(memory_space=pl.ANY)
    out = pl.pallas_call(
        lambda *refs: _kernel(*refs, M=M, D=D),
        in_specs=[any_spec] * 4,
        out_specs=any_spec,
        out_shape=jax.ShapeDtypeStruct((M, D), x.dtype),
        scratch_shapes=[
            pltpu.VMEM((M, D), jnp.bfloat16),
            pltpu.VMEM((NT, D, _BLK), jnp.bfloat16),
            pltpu.VMEM((NT, M + 2 * _BLK, _BLK), jnp.bfloat16),
            pltpu.VMEM((D,), jnp.bfloat16),
            pltpu.VMEM((D,), jnp.bfloat16),
            pltpu.VMEM((8, D), jnp.float32),
            pltpu.SemaphoreType.DMA((NB + NT + 2,)),
            pltpu.SemaphoreType.DMA,
        ],
        compiler_params=pltpu.CompilerParams(vmem_limit_bytes=64 << 20),
    )(x.reshape(M, D), g, b, w)
    return out.reshape(B, S, D)
```

```python
import jax
import jax.numpy as jnp
from jax import lax
import jax.experimental.pallas as pl
import jax.experimental.pallas.tpu as pltpu

_EPS = 1e-5
_BLK = 128
_GRP = 16
_P = 4
_U = 4


def _num_x_sems(NB):
    return _P + 2 + pl.cdiv(NB - _P - 2, _U)


def _kernel(x_hbm, g_hbm, b_hbm, w_hbm, o_hbm,
            xo, wbuf, ybuf, g16, b16, gb, sem_in, sem_o, *, M, D):
    NB = M // _BLK
    NT = D // _BLK
    NS = _num_x_sems(NB)
    GPB = _BLK // _GRP
    y32 = ybuf.bitcast(jnp.uint32)
    w32 = wbuf.bitcast(jnp.uint32)
    LASTQ = GPB * NB - 1
    DUMMYQ = GPB * NB + GPB

    def xcopy(i):
        r = pl.multiple_of(i * _BLK, _BLK)
        return pltpu.make_async_copy(
            x_hbm.at[pl.ds(r, _BLK), :], xo.at[pl.ds(r, _BLK), :], sem_in.at[i])

    NC = (NB - _P - 2) // _U
    TAIL = (NB - _P - 2) % _U

    def ccopy(c, nblk=_U):
        r = pl.multiple_of((_P + 2 + c * _U) * _BLK, _BLK)
        return pltpu.make_async_copy(
            x_hbm.at[pl.ds(r, nblk * _BLK), :], xo.at[pl.ds(r, nblk * _BLK), :],
            sem_in.at[_P + 2 + c])

    def wcopy(j):
        c = pl.multiple_of(j * _BLK, _BLK)
        return pltpu.make_async_copy(
            w_hbm.at[:, pl.ds(c, _BLK)], wbuf.at[j], sem_in.at[NS + j])

    def gcopy():
        return pltpu.make_async_copy(g_hbm, g16, sem_in.at[NS + NT])

    def bcopy():
        return pltpu.make_async_copy(b_hbm, b16, sem_in.at[NS + NT + 1])

    def ocopy(i, nt):
        r = pl.multiple_of(i * _BLK, _BLK)
        c = pl.multiple_of(nt * _BLK, _BLK)
        return pltpu.make_async_copy(
            xo.at[pl.ds(r, _BLK), pl.ds(c, _BLK)],
            o_hbm.at[pl.ds(r, _BLK), pl.ds(c, _BLK)], sem_o)

    def ln_load(q):
        return xo[pl.ds(pl.multiple_of(q * _GRP, _GRP), _GRP), :]

    def ln_stats(q):
        x = ln_load(q).astype(jnp.float32)
        mean = jnp.mean(x, axis=-1, keepdims=True)
        xc = x - mean
        var = jnp.mean(xc * xc, axis=-1, keepdims=True)
        rstd = lax.rsqrt(var + _EPS)
        return (jnp.broadcast_to(rstd, (_GRP, _BLK)),
                jnp.broadcast_to(mean, (_GRP, _BLK)))

    def ln_apply(q, xb, stats):
        rstd, mean = stats
        yv = ybuf.at[:, pl.ds(pl.multiple_of(q * _GRP, _GRP), _GRP), :]
        x = xb.astype(jnp.float32)
        for kt in range(NT):
            cols = slice(kt * _BLK, (kt + 1) * _BLK)
            y = (x[:, cols] - mean) * rstd * gb[0:1, cols] + gb[1:2, cols]
            yv[kt] = y.astype(jnp.bfloat16)

    def ln_block(blk):
        for grp in range(GPB):
            q = GPB * blk + grp
            ln_apply(q, ln_load(q), ln_stats(q))

    def step(blk, nt, mid=None, post=None):
        yv = y32.at[:, pl.ds(pl.multiple_of(blk * (_BLK // 2), _BLK // 2), _BLK // 2), :]
        lhs = jnp.concatenate(
            [pltpu.bitcast(yv[kt], jnp.bfloat16) for kt in range(NT)], axis=1)
        rhs = pltpu.bitcast(w32[nt], jnp.bfloat16)
        acc = jnp.dot(lhs, rhs, preferred_element_type=jnp.float32)
        held = mid() if mid is not None else None
        ov = xo.at[pl.ds(pl.multiple_of(blk * _BLK, _BLK), _BLK), :]
        ov[:, pl.ds(pl.multiple_of(nt * _BLK, _BLK), _BLK)] = acc.astype(jnp.bfloat16)
        ocopy(blk, nt).start()
        if post is not None:
            post(held)
        return held

    def ln_step(blk, nt, q_apply_load, q_apply_store, q_stats, stats):
        held = step(
            blk, nt,
            mid=lambda: (ln_load(q_apply_load), ln_stats(q_stats)),
            post=lambda h: ln_apply(q_apply_store, h[0], stats))
        return held[1]

    nslots = GPB + 1
    s0 = (NT - 1) * _P - nslots
    nt0 = 1 + s0 // _P
    xcopy(0).start()
    gcopy().start()
    bcopy().start()
    wcopy(0).start()
    for i in range(1, _P):
        xcopy(i).start()
    for j in range(1, NT):
        if j == nt0 + 1:
            xcopy(_P).start()
        wcopy(j).start()
    xcopy(_P + 1).start()
    ccopy(0).start()
    ccopy(1).start()

    xcopy(0).wait()
    gcopy().wait()
    bcopy().wait()
    gb[0:1, :] = g16[...].astype(jnp.float32).reshape(1, D)
    gb[1:2, :] = b16[...].astype(jnp.float32).reshape(1, D)
    ln_block(0)
    wcopy(0).wait()
    for i in range(_P):
        if i > 0:
            xcopy(i).wait()
            ln_block(i)
        step(i, 0)

    def startup_slab(nt, stats):
        for i in range(_P):
            s = (nt - 1) * _P + i - s0
            act = s >= 0
            stats = ln_step(
                i, nt,
                jnp.where(act, GPB * _P + s, 0),
                jnp.where(act, GPB * _P + s, DUMMYQ),
                jnp.where(s + 1 >= 0, jnp.minimum(GPB * _P + s + 1, GPB * _P + GPB), 0),
                stats)
        return stats

    def startup(p, stats):
        nt = 1 + 2 * p
        wcopy(nt).wait()
        wcopy(nt + 1).wait()

        @pl.when(p == (nt0 - 1) // 2)
        def _():
            xcopy(_P).wait()

        return startup_slab(nt + 1, startup_slab(nt, stats))

    zero = jnp.zeros((_GRP, _BLK), jnp.float32)
    stats = lax.fori_loop(0, (NT - 2) // 2, startup, (zero, zero))
    wcopy(NT - 1).wait()
    xcopy(_P + 1).wait()
    startup_slab(NT - 1, stats)

    def main(j, stats):
        b0 = _P + j * _U
        @pl.when(j < NC)
        def _():
            ccopy(j).wait()

        @pl.when(j == NC)
        def _():
            ccopy(NC, TAIL).wait()

        @pl.when(j + 2 < NC)
        def _():
            ccopy(j + 2).start()

        @pl.when(j + 2 == NC)
        def _():
            ccopy(NC, TAIL).start()

        for k in range(_U):
            blk = b0 + k
            for nt in range(NT):
                q = GPB * (blk + 1) + nt + 1
                stats = ln_step(blk, nt, jnp.minimum(q, LASTQ), q,
                                jnp.minimum(q + 1, LASTQ), stats)
        return stats

    lax.fori_loop(0, (NB - _P) // _U, main, ln_stats(GPB * (_P + 1) + 1))

    pltpu.make_async_copy(xo, o_hbm, sem_o).wait()


@jax.jit
def pallas_standalone__layernorm_linear__prompt_kernel(
    x: jax.Array,
    g: jax.Array,
    b: jax.Array,
    w: jax.Array,
):
    B, S, D = x.shape
    M = B * S
    NB = M // _BLK
    NT = D // _BLK
    any_spec = pl.BlockSpec(memory_space=pl.ANY)
    out = pl.pallas_call(
        lambda *refs: _kernel(*refs, M=M, D=D),
        in_specs=[any_spec] * 4,
        out_specs=any_spec,
        out_shape=jax.ShapeDtypeStruct((M, D), x.dtype),
        scratch_shapes=[
            pltpu.VMEM((M, D), jnp.bfloat16),
            pltpu.VMEM((NT, D, _BLK), jnp.bfloat16),
            pltpu.VMEM((NT, M + 2 * _BLK, _BLK), jnp.bfloat16),
            pltpu.VMEM((D,), jnp.bfloat16),
            pltpu.VMEM((D,), jnp.bfloat16),
            pltpu.VMEM((8, D), jnp.float32),
            pltpu.SemaphoreType.DMA((_num_x_sems(NB) + NT + 2,)),
            pltpu.SemaphoreType.DMA,
        ],
        compiler_params=pltpu.CompilerParams(
            vmem_limit_bytes=64 << 20,
            disable_bounds_checks=True,
            disable_semaphore_checks=True),
    )(x.reshape(M, D), g, b, w)
    return out.reshape(B, S, D)
```

```python
import jax
import jax.numpy as jnp
from jax import lax
import jax.experimental.pallas as pl
import jax.experimental.pallas.tpu as pltpu

_EPS = 1e-5
_BLK = 128
_GRP = 16
_P = 4
_U = 4


def _num_x_sems(NB):
    return _P + 2 + pl.cdiv(NB - _P - 2, _U)


def _kernel(x_hbm, g_hbm, b_hbm, w_hbm, o_hbm,
            xo, wbuf, ybuf, g16, b16, gb, sem_in, sem_o, *, M, D):
    NB = M // _BLK
    NT = D // _BLK
    NS = _num_x_sems(NB)
    GPB = _BLK // _GRP
    y32 = ybuf.bitcast(jnp.uint32)
    w32 = wbuf.bitcast(jnp.uint32)
    LASTQ = GPB * NB - 1
    DUMMYQ = GPB * NB + GPB

    def xcopy(i):
        r = pl.multiple_of(i * _BLK, _BLK)
        return pltpu.make_async_copy(
            x_hbm.at[pl.ds(r, _BLK), :], xo.at[pl.ds(r, _BLK), :], sem_in.at[i])

    NC = (NB - _P - 2) // _U
    TAIL = (NB - _P - 2) % _U

    def ccopy(c, nblk=_U):
        r = pl.multiple_of((_P + 2 + c * _U) * _BLK, _BLK)
        return pltpu.make_async_copy(
            x_hbm.at[pl.ds(r, nblk * _BLK), :], xo.at[pl.ds(r, nblk * _BLK), :],
            sem_in.at[_P + 2 + c])

    def wcopy(j):
        c = pl.multiple_of(j * _BLK, _BLK)
        return pltpu.make_async_copy(
            w_hbm.at[:, pl.ds(c, _BLK)], wbuf.at[j], sem_in.at[NS + j])

    def gcopy():
        return pltpu.make_async_copy(g_hbm, g16, sem_in.at[NS + NT])

    def bcopy():
        return pltpu.make_async_copy(b_hbm, b16, sem_in.at[NS + NT + 1])

    def ocopy(i, nt):
        r = pl.multiple_of(i * _BLK, _BLK)
        c = pl.multiple_of(nt * _BLK, _BLK)
        return pltpu.make_async_copy(
            xo.at[pl.ds(r, _BLK), pl.ds(c, _BLK)],
            o_hbm.at[pl.ds(r, _BLK), pl.ds(c, _BLK)], sem_o)

    def ln_load(q):
        return xo[pl.ds(pl.multiple_of(q * _GRP, _GRP), _GRP), :]

    def ln_stats(q):
        x = ln_load(q).astype(jnp.float32)
        mean = jnp.mean(x, axis=-1, keepdims=True)
        xc = x - mean
        var = jnp.mean(xc * xc, axis=-1, keepdims=True)
        rstd = lax.rsqrt(var + _EPS)
        return (jnp.broadcast_to(rstd, (_GRP, _BLK)),
                jnp.broadcast_to(mean, (_GRP, _BLK)))

    def ln_apply(q, xb, stats):
        rstd, mean = stats
        yv = ybuf.at[:, pl.ds(pl.multiple_of(q * _GRP, _GRP), _GRP), :]
        x = xb.astype(jnp.float32)
        for kt in range(NT):
            cols = slice(kt * _BLK, (kt + 1) * _BLK)
            y = (x[:, cols] - mean) * rstd * gb[0:1, cols] + gb[1:2, cols]
            yv[kt] = y.astype(jnp.bfloat16)

    def ln_block(blk):
        for grp in range(GPB):
            q = GPB * blk + grp
            x = ln_load(q).astype(jnp.float32)
            mean = jnp.mean(x, axis=-1, keepdims=True)
            xc = x - mean
            var = jnp.mean(xc * xc, axis=-1, keepdims=True)
            xn = xc * lax.rsqrt(var + _EPS)
            yv = ybuf.at[:, pl.ds(q * _GRP, _GRP), :]
            for kt in range(NT):
                cols = slice(kt * _BLK, (kt + 1) * _BLK)
                y = xn[:, cols] * gb[0:1, cols] + gb[1:2, cols]
                yv[kt] = y.astype(jnp.bfloat16)

    def step(blk, nt, mid=None, post=None):
        yv = y32.at[:, pl.ds(pl.multiple_of(blk * (_BLK // 2), _BLK // 2), _BLK // 2), :]
        lhs = jnp.concatenate(
            [pltpu.bitcast(yv[kt], jnp.bfloat16) for kt in range(NT)], axis=1)
        rhs = pltpu.bitcast(w32[nt], jnp.bfloat16)
        acc = jnp.dot(lhs, rhs, preferred_element_type=jnp.float32)
        held = mid() if mid is not None else None
        ov = xo.at[pl.ds(pl.multiple_of(blk * _BLK, _BLK), _BLK), :]
        ov[:, pl.ds(pl.multiple_of(nt * _BLK, _BLK), _BLK)] = acc.astype(jnp.bfloat16)
        ocopy(blk, nt).start()
        if post is not None:
            post(held)
        return held

    def ln_step(blk, nt, q_apply_load, q_apply_store, q_stats, stats):
        held = step(
            blk, nt,
            mid=lambda: (ln_load(q_apply_load), ln_stats(q_stats)),
            post=lambda h: ln_apply(q_apply_store, h[0], stats))
        return held[1]

    nslots = GPB + 1
    s0 = (NT - 1) * _P - nslots
    nt0 = 1 + s0 // _P
    xcopy(0).start()
    gcopy().start()
    bcopy().start()
    wcopy(0).start()
    for i in range(1, _P):
        xcopy(i).start()
    for j in range(1, NT):
        if j == nt0 + 1:
            xcopy(_P).start()
        wcopy(j).start()
    xcopy(_P + 1).start()
    ccopy(0).start()
    ccopy(1).start()

    xcopy(0).wait()
    gcopy().wait()
    bcopy().wait()
    gb[0:1, :] = g16[...].astype(jnp.float32).reshape(1, D)
    gb[1:2, :] = b16[...].astype(jnp.float32).reshape(1, D)
    ln_block(0)
    wcopy(0).wait()
    for i in range(_P):
        if i > 0:
            xcopy(i).wait()
            ln_block(i)
        step(i, 0)

    def startup_slab(nt, stats):
        for i in range(_P):
            s = (nt - 1) * _P + i - s0
            act = s >= 0
            stats = ln_step(
                i, nt,
                jnp.where(act, GPB * _P + s, 0),
                jnp.where(act, GPB * _P + s, DUMMYQ),
                jnp.where(s + 1 >= 0, jnp.minimum(GPB * _P + s + 1, GPB * _P + GPB), 0),
                stats)
        return stats

    def startup(p, stats):
        nt = 1 + 2 * p
        wcopy(nt).wait()
        wcopy(nt + 1).wait()

        @pl.when(p == (nt0 - 1) // 2)
        def _():
            xcopy(_P).wait()

        return startup_slab(nt + 1, startup_slab(nt, stats))

    zero = jnp.zeros((_GRP, _BLK), jnp.float32)
    stats = lax.fori_loop(0, (NT - 2) // 2, startup, (zero, zero))
    wcopy(NT - 1).wait()
    xcopy(_P + 1).wait()
    startup_slab(NT - 1, stats)

    def main(j, stats):
        b0 = _P + j * _U
        @pl.when(j < NC)
        def _():
            ccopy(j).wait()

        @pl.when(j == NC)
        def _():
            ccopy(NC, TAIL).wait()

        @pl.when(j + 2 < NC)
        def _():
            ccopy(j + 2).start()

        @pl.when(j + 2 == NC)
        def _():
            ccopy(NC, TAIL).start()

        for k in range(_U):
            blk = b0 + k
            for nt in range(NT):
                q = GPB * (blk + 1) + nt + 1
                stats = ln_step(blk, nt, jnp.minimum(q, LASTQ), q,
                                jnp.minimum(q + 1, LASTQ), stats)
        return stats

    lax.fori_loop(0, (NB - _P) // _U, main, ln_stats(GPB * (_P + 1) + 1))

    pltpu.make_async_copy(xo, o_hbm, sem_o).wait()


@jax.jit
def pallas_standalone__layernorm_linear__prompt_kernel(
    x: jax.Array,
    g: jax.Array,
    b: jax.Array,
    w: jax.Array,
):
    B, S, D = x.shape
    M = B * S
    NB = M // _BLK
    NT = D // _BLK
    any_spec = pl.BlockSpec(memory_space=pl.ANY)
    out = pl.pallas_call(
        lambda *refs: _kernel(*refs, M=M, D=D),
        in_specs=[any_spec] * 4,
        out_specs=any_spec,
        out_shape=jax.ShapeDtypeStruct((M, D), x.dtype),
        scratch_shapes=[
            pltpu.VMEM((M, D), jnp.bfloat16),
            pltpu.VMEM((NT, D, _BLK), jnp.bfloat16),
            pltpu.VMEM((NT, M + 2 * _BLK, _BLK), jnp.bfloat16),
            pltpu.VMEM((D,), jnp.bfloat16),
            pltpu.VMEM((D,), jnp.bfloat16),
            pltpu.VMEM((8, D), jnp.float32),
            pltpu.SemaphoreType.DMA((_num_x_sems(NB) + NT + 2,)),
            pltpu.SemaphoreType.DMA,
        ],
        compiler_params=pltpu.CompilerParams(
            vmem_limit_bytes=64 << 20,
            disable_bounds_checks=True,
            disable_semaphore_checks=True),
    )(x.reshape(M, D), g, b, w)
    return out.reshape(B, S, D)
```
